```python
import jax
import jax.numpy as jnp

def _softmax(x, axis=-1):
    return jax.nn.softmax(x, axis=axis)

def _gelu(x):
    return jax.nn.gelu(x, approximate=True)

def _silu(x):
    return jax.nn.silu(x)

def _sigmoid(x):
    return jax.nn.sigmoid(x)

def _layernorm(x, axis=-1, eps=1e-05):
    m = jnp.mean(x, axis=axis, keepdims=True)
    v = jnp.var(x, axis=axis, keepdims=True)
    return (x - m) / jnp.sqrt(v + eps)

def _scatter_add(tgt, idx, src, axis=0):
    return tgt.at[idx].add(src)

def _segment_sum(src, seg, n):
    return jax.ops.segment_sum(src, seg, n)

class _Rng:

    def __init__(self, key):
        self._k = key

    def _next(self):
        self._k, sub = jax.random.split(self._k)
        return sub

    def normal(self, shape):
        return jax.random.normal(self._next(), shape, dtype=jnp.bfloat16)

    def randint(self, lo, hi, shape):
        return jax.random.randint(self._next(), shape, lo, hi, dtype=jnp.int32)

    def uniform(self, shape, lo=0.0, hi=1.0):
        return jax.random.uniform(self._next(), shape, jnp.bfloat16, lo, hi)

    def permutation(self, n):
        return jax.random.permutation(self._next(), n)
kernel_name = 'adaLN_cond__sliding_block_cached__dense_activation_mish__decode'

def setup_inputs():
    _rng = _Rng(jax.random.key(int.from_bytes(__import__("os").urandom(4), "little")))
    _w = lambda a: (lambda t: t.astype(jnp.bfloat16) if jnp.issubdtype(t.dtype, jnp.floating) else t)(jnp.asarray(a))

    def _A_setup():
        B, Sq, D = (1, 1, 640)
        Hq, Hkv, Sk, Dh = (32, 32, 32768, 192)
        assert Hq % Hkv == 0, (Hq, Hkv)
        return {'x': _w((lambda *s: _rng.normal(s) * 0.05)(B, Sq, D)), 'k_cache': _w((lambda *s: _rng.normal(s) * 0.05)(B, Hkv, Sk, Dh)), 'v_cache': _w((lambda *s: _rng.normal(s) * 0.05)(B, Hkv, Sk, Dh)), 'wq': _w((lambda *s: _rng.normal(s) * 0.05)(D, Hq * Dh) * D ** (-0.5)), 'wo': _w((lambda *s: _rng.normal(s) * 0.05)(Hq * Dh, D) * (Hq * Dh) ** (-0.5))}
    _A_in = _A_setup()

    def _B_setup():
        B, S, D, F = (1, 1, 640, 1536)
        return {'x': _w((lambda *s: _rng.normal(s) * 0.05)(B, S, D)), 'w1': _w((lambda *s: _rng.normal(s) * 0.05)(D, F) * D ** (-0.5)), 'b1': _w((lambda *s: _rng.normal(s) * 0.05)(F)), 'w2': _w((lambda *s: _rng.normal(s) * 0.05)(F, D) * F ** (-0.5))}
    _B_in = _B_setup()
    return {'A_x': _A_in['x'], 'A_k_cache': _A_in['k_cache'], 'A_v_cache': _A_in['v_cache'], 'A_wq': _A_in['wq'], 'A_wo': _A_in['wo'], 'B_x': _B_in['x'], 'B_w1': _B_in['w1'], 'B_b1': _B_in['b1'], 'B_w2': _B_in['w2'], 'c': _w((lambda *s: _rng.normal(s) * 0.05)(1, 640)), 'w_mod': _w((lambda *s: _rng.normal(s) * 0.05)(640, 6 * 640) * 640 ** (-0.5))}

def reference(A_x, A_k_cache, A_v_cache, A_wq, A_wo, B_x, B_w1, B_b1, B_w2, c, w_mod):

    def _A_ref(x, k_cache, v_cache, wq, wo):
        B, Sq, D = x.shape
        Hq, Dh = (32, 192)
        Hkv, Sk = (k_cache.shape[1], k_cache.shape[2])
        W = min(4096, max(256, Sk // 4))
        rep = Hq // Hkv
        q = (lambda x, *d: x.transpose(*d))((x @ wq).reshape(B, Sq, Hq, Dh), 0, 2, 1, 3)
        k = jnp.repeat(k_cache[:, :, Sk - W:, :], rep, axis=1)
        v = jnp.repeat(v_cache[:, :, Sk - W:, :], rep, axis=1)
        scores = jnp.einsum('bhqd,bhkd->bhqk', q, k) * Dh ** (-0.5)
        p = _softmax(scores, axis=-1)
        o = jnp.einsum('bhqk,bhkd->bhqd', p, v)
        return (lambda x, *d: x.transpose(*d))(o, 0, 2, 1, 3).reshape(B, Sq, Hq * Dh) @ wo

    def _B_ref(x, w1, b1, w2):
        h = jnp.einsum('bsd,df->bsf', x, w1) + b1
        sp = jnp.log1p(jnp.exp(-jnp.abs(h))) + jnp.where(h > 0, h, jnp.zeros_like(h))
        act = h * jnp.tanh(sp)
        return jnp.einsum('bsf,fd->bsd', act, w2)
    x = A_x
    mod = (_silu(c) @ w_mod).reshape(c.shape[0], 6, 1, -1)
    sa, ca, ga, sb, cb, gb = (mod[:, 0].copy(), mod[:, 1].copy(), mod[:, 2].copy(), mod[:, 3].copy(), mod[:, 4].copy(), mod[:, 5].copy())
    h = _layernorm(x, axis=-1) * (1 + ca) + sa
    x = x + ga * _A_ref(h, A_k_cache, A_v_cache, A_wq, A_wo)
    h = _layernorm(x, axis=-1) * (1 + cb) + sb
    x = x + gb * _B_ref(h, B_w1, B_b1, B_w2)
    return x
```

```python
import functools

import jax
import jax.numpy as jnp
from jax import lax
from jax.experimental import pallas as pl
from jax.experimental.pallas import tpu as pltpu

F32 = jnp.float32
BF16 = jnp.bfloat16
LANES = 128
SUB = 8


def _tree_sum(xs):
    xs = list(xs)
    while len(xs) > 1:
        xs = [xs[i] + xs[i + 1] if i + 1 < len(xs) else xs[i] for i in range(0, len(xs), 2)]
    return xs[0]


def _layernorm(x, eps=1e-5):
    m = jnp.mean(x, axis=-1, keepdims=True)
    d = x - m
    v = jnp.mean(d * d, axis=-1, keepdims=True)
    return d / jnp.sqrt(v + eps)


def _make(L0=16, L1=24, S=32, delay=0, nobc=True, fine=False, start_delay=0, f2_lumps=4, compute=True):
    LAG = (L0, L1)
    assert S & (S - 1) == 0

    def fn(A_x, A_k_cache, A_v_cache, A_wq, A_wo, B_x, B_w1, B_b1, B_w2, c, w_mod):
        del B_x
        D = A_x.shape[-1]
        _, H, SK, DH = A_k_cache.shape
        W = min(4096, max(256, SK // 4))
        F = B_w1.shape[1]
        NM = w_mod.shape[1]
        HD = H * DH
        QB = 2048
        n_m = D // SUB
        n_q = D // (2 * SUB)
        n_qb = HD // QB
        n_kv = DH // SUB
        RO = 24
        n_o = HD // (2 * RO)
        n_f1 = D // (2 * SUB)
        n_f2 = F // (2 * RO)
        base_q = n_m
        base_h = base_q + n_q * n_qb
        base_o = base_h + 2 * n_kv * H
        base_f1 = base_o + n_o
        base_f2 = base_f1 + n_f1
        assert max(LAG) <= min(n_kv, S)
        scale = float(DH) ** -0.5

        def kernel(x_hbm, k_hbm, v_hbm, wq_hbm, wo_hbm, w1_hbm, b1_hbm, w2_hbm, c_hbm, wm_hbm,
                   o_ref,
                   wm_v, wq_v, k_v, v_v, wo_v, w1_v, w2_v, x_v, c_v, b1_v,
                   row_v, col_v, q_v, s_v, ob_v, sems, small_sems):

            def sem(t, step):
                return sems.at[t, step & (S - 1)]

            def cp_m(t, i):
                cols = pl.ds(t * (NM // 2), NM // 2)
                return pltpu.make_async_copy(wm_hbm.at[i, :, cols], wm_v.at[i, :, cols], sem(t, i))

            def cp_q(t, cb, r):
                cols = pl.ds(pl.multiple_of(cb * QB, QB), QB)
                return pltpu.make_async_copy(wq_hbm.at[r, t, :, cols], wq_v.at[cb, r, t],
                                             sem(t, base_q + cb * n_q + r))

            def cp_kv(src, dst, which, h, t, i):
                half = W // 2
                return pltpu.make_async_copy(
                    src.at[h * n_kv + i, :, pl.ds(SK - W + t * half, half)],
                    dst.at[i, :, pl.ds(t * half, half)],
                    sem(t, base_h + (2 * h + which) * n_kv + i))

            cp_k = functools.partial(cp_kv, k_hbm, k_v, 0)
            cp_v = functools.partial(cp_kv, v_hbm, v_v, 1)

            def cp_rows(src, dst, base, t, i):
                return pltpu.make_async_copy(src.at[i, t], dst.at[i, t], sem(t, base + i))

            cp_o = functools.partial(cp_rows, wo_hbm, wo_v, base_o)
            cp_f1 = functools.partial(cp_rows, w1_hbm, w1_v, base_f1)
            cp_f2 = functools.partial(cp_rows, w2_hbm, w2_v, base_f2)

            def start(cp):
                return lambda t, *i: cp(t, *i).start(priority=t)

            def advance(wait, start_ahead):
                if fine:
                    for t in (0, 1):
                        wait(t)
                        start_ahead(t)
                else:
                    for t in (0, 1):
                        wait(t)
                    for t in (0, 1):
                        start_ahead(t)
                if delay:
                    pl.delay(delay)

            def flat(n, cp, start_next):
                def step(i):
                    def start_ahead(t):
                        nxt = i + LAG[t]
                        pl.when(nxt < n)(lambda: start(cp)(t, nxt))
                        if start_next is not None:
                            pl.when(nxt >= n)(lambda: start_next(t, nxt - n))
                    advance(lambda t: cp(t, i).wait(), start_ahead)
                return step

            def put_cols(v):
                for j in range(v.shape[1] // LANES):
                    t = jnp.broadcast_to(v[:, j * LANES:(j + 1) * LANES], (LANES, LANES)).T
                    for g in range(LANES // SUB):
                        col_v[j * (LANES // SUB) + g] = t[g * SUB:(g + 1) * SUB]

            def scaled(w, col):
                w = w.astype(F32)
                return w * jnp.tile(col, (1, w.shape[1] // LANES))

            def matvec(lo, hi, step, tiles, acc):
                def body(i, acc):
                    step(i)
                    if not compute:
                        return acc
                    return acc + _tree_sum(scaled(w, col) for w, col in tiles(i))
                return lax.fori_loop(lo, hi, body, acc)

            def matvec_wide(n, width, step, tile):
                s_v[:, :width] = jnp.zeros((SUB, width), F32)

                def body(i, _):
                    step(i)
                    if compute:
                        s_v[:, :width] += scaled(*tile(i))
                lax.fori_loop(0, n, body, None)
                return jnp.sum(s_v[:, :width], axis=0, keepdims=True)

            cp_c = pltpu.make_async_copy(c_hbm, c_v, small_sems.at[0])
            cp_x = pltpu.make_async_copy(x_hbm, x_v, small_sems.at[1])
            cp_b = pltpu.make_async_copy(b1_hbm, b1_v, small_sems.at[2])
            cp_c.start()
            for i in range(max(LAG)):
                for t in (0, 1):
                    if i < LAG[t]:
                        start(cp_m)(t, i)
                if start_delay and i < LAG[0]:
                    pl.delay(start_delay)
            cp_x.start()
            cp_b.start()

            cp_c.wait()
            cf = c_v[...].astype(F32)
            put_cols(cf * jax.nn.sigmoid(cf))
            mod = matvec_wide(n_m, NM, flat(n_m, cp_m, lambda t, i: start(cp_q)(t, 0, i)),
                              lambda i: (wm_v[i], col_v[i]))
            sa, ca, ga, sb, cb_, gb = (mod[:, j * D:(j + 1) * D] for j in range(6))
            cp_x.wait()
            x = x_v[0].astype(F32)
            put_cols(_layernorm(x) * (1.0 + ca) + sa)

            def q_block(cb, _):
                def step(r):
                    def start_ahead(t):
                        nxt = r + LAG[t]
                        wrap = (nxt >= n_q).astype(jnp.int32)
                        ncb, nr = cb + wrap, nxt - wrap * n_q
                        pl.when(ncb < n_qb)(lambda: start(cp_q)(t, ncb, nr))
                        pl.when(ncb == n_qb)(lambda: start(functools.partial(cp_k, 0))(t, nr))
                    advance(lambda t: cp_q(t, cb, r).wait(), start_ahead)
                q = matvec(0, n_q, step, lambda r: [(wq_v[cb, r, t], col_v[2 * r + t]) for t in (0, 1)],
                           jnp.zeros((SUB, QB), F32))
                q = jnp.sum(q, axis=0, keepdims=True) * scale
                for j in range(QB // LANES):
                    q_v[cb * (QB // LANES) + j] = jnp.broadcast_to(q[:, j * LANES:(j + 1) * LANES], (SUB, LANES))
            lax.fori_loop(0, n_qb, q_block, None)

            diag = (lax.broadcasted_iota(jnp.int32, (SUB, LANES), 1)
                    - lax.broadcasted_iota(jnp.int32, (SUB, LANES), 0))

            def lane_sum(v):
                return jnp.broadcast_to(jnp.sum(v, axis=1, keepdims=True), (SUB, LANES))

            def q_cols(h):
                for i in range(n_kv):
                    g = h * n_kv + i
                    col_v[i] = lane_sum(jnp.where(diag == (g & 15) * SUB, q_v[g >> 4], 0.0))

            q_cols(0)

            def head(h, _):
                s = matvec_wide(n_kv, W, flat(n_kv, functools.partial(cp_k, h), start(functools.partial(cp_v, h))),
                                lambda i: (k_v[i], col_v[i]))
                e = jnp.exp(s - jnp.max(s, axis=1, keepdims=True))
                s_v[...] = jnp.broadcast_to(e, (SUB, W))
                denom = _tree_sum(e[:, j * LANES:(j + 1) * LANES] for j in range(W // LANES))

                def start_next(t, i):
                    pl.when(h + 1 < H)(lambda: start(functools.partial(cp_k, h + 1))(t, i))
                    pl.when(h + 1 == H)(lambda: start(cp_o)(t, i))

                step = flat(n_kv, functools.partial(cp_v, h), start_next)

                def pv(i, _):
                    step(i)
                    if compute:
                        prod = v_v[i].astype(F32) * s_v[...]
                        ob_v[h * n_kv + i] = _tree_sum(prod[:, j * LANES:(j + 1) * LANES] for j in range(W // LANES))
                lax.fori_loop(0, n_kv, pv, None)

                inv = 1.0 / lane_sum(jnp.broadcast_to(denom, (SUB, LANES)))
                for i in range(n_kv):
                    ob_v[h * n_kv + i] = lane_sum(ob_v[h * n_kv + i]) * inv
                q_cols(jnp.minimum(h + 1, H - 1))
            lax.fori_loop(0, H, head, None)

            def tall(ref, cols):
                per = RO // SUB
                return lambda i: [(ref[i, t, pl.ds(r * SUB, SUB), :], cols(i, t * per + r))
                                  for t in (0, 1) for r in range(per)]
            gps = 2 * RO // SUB
            attn = matvec(0, n_o, flat(n_o, cp_o, start(cp_f1)), tall(wo_v, lambda i, j: ob_v[i * gps + j]),
                          jnp.zeros((SUB, D), F32))
            x1 = x + ga * jnp.sum(attn, axis=0, keepdims=True)
            put_cols(_layernorm(x1) * (1.0 + cb_) + sb)

            a = matvec(0, n_f1, flat(n_f1, cp_f1, start(cp_f2)),
                       lambda i: [(w1_v[i, t], col_v[2 * i + t]) for t in (0, 1)], jnp.zeros((SUB, F), F32))
            cp_b.wait()
            a = jnp.sum(a, axis=0, keepdims=True) + b1_v[...].astype(F32).reshape(1, F)
            sp = jnp.log1p(jnp.exp(-jnp.abs(a))) + jnp.where(a > 0, a, 0.0)
            act = a * jnp.tanh(sp)
            fl = F // f2_lumps
            for j in range(f2_lumps):
                row_v[j] = act[:, j * fl:(j + 1) * fl]
            n_l = n_f2 // f2_lumps

            def lump(j, y):
                put_cols(row_v[j])
                return matvec(j * n_l, (j + 1) * n_l, flat(n_f2, cp_f2, None),
                              tall(w2_v, lambda i, r: col_v[(i - j * n_l) * gps + r]), y)
            y = lax.fori_loop(0, f2_lumps, lump, jnp.zeros((SUB, D), F32))
            o_ref[0] = (x1 + gb * jnp.sum(y, axis=0, keepdims=True)).astype(o_ref.dtype)

        any_spec = pl.BlockSpec(memory_space=pl.ANY)
        kt = jnp.swapaxes(A_k_cache, 2, 3).reshape(H * n_kv, SUB, SK)
        vt = jnp.swapaxes(A_v_cache, 2, 3).reshape(H * n_kv, SUB, SK)
        return pl.pallas_call(
            kernel,
            out_shape=jax.ShapeDtypeStruct(A_x.shape, A_x.dtype),
            in_specs=[any_spec] * 10,
            out_specs=pl.BlockSpec(memory_space=pltpu.VMEM),
            scratch_shapes=[
                pltpu.VMEM((n_m, SUB, NM), BF16),
                pltpu.VMEM((n_qb, n_q, 2, SUB, QB), BF16),
                pltpu.VMEM((n_kv, SUB, W), BF16),
                pltpu.VMEM((n_kv, SUB, W), BF16),
                pltpu.VMEM((n_o, 2, RO, D), BF16),
                pltpu.VMEM((n_f1, 2, SUB, F), BF16),
                pltpu.VMEM((n_f2, 2, RO, D), BF16),
                pltpu.VMEM(A_x.shape, BF16),
                pltpu.VMEM(c.shape, BF16),
                pltpu.VMEM(B_b1.shape, BF16),
                pltpu.VMEM((f2_lumps, 1, F // f2_lumps), F32),
                pltpu.VMEM((max(D, F // f2_lumps) // SUB, SUB, LANES), F32),
                pltpu.VMEM((HD // LANES, SUB, LANES), F32),
                pltpu.VMEM((SUB, W), F32),
                pltpu.VMEM((HD // SUB, SUB, LANES), F32),
                pltpu.SemaphoreType.DMA((2, S)),
                pltpu.SemaphoreType.DMA((3,)),
            ],
            compiler_params=pltpu.CompilerParams(vmem_limit_bytes=64 * 1024 * 1024, disable_bounds_checks=nobc),
        )(A_x, kt, vt, A_wq.reshape(n_q, 2, SUB, HD), A_wo.reshape(n_o, 2, RO, D),
          B_w1.reshape(n_f1, 2, SUB, F), B_b1, B_w2.reshape(n_f2, 2, RO, D), c,
          w_mod.reshape(n_m, SUB, NM))

    return fn


@jax.jit
def pallas_adaLN_cond__sliding_block_cached__dense_activation_mish__decode_kernel(
    A_x: jax.Array,
    A_k_cache: jax.Array,
    A_v_cache: jax.Array,
    A_wq: jax.Array,
    A_wo: jax.Array,
    B_x: jax.Array,
    B_w1: jax.Array,
    B_b1: jax.Array,
    B_w2: jax.Array,
    c: jax.Array,
    w_mod: jax.Array,
):
    return _make()(A_x, A_k_cache, A_v_cache, A_wq, A_wo, B_x, B_w1, B_b1, B_w2, c, w_mod)
```

```python
import functools

import jax
import jax.numpy as jnp
from jax import lax
from jax.experimental import pallas as pl
from jax.experimental.pallas import tpu as pltpu

F32 = jnp.float32
BF16 = jnp.bfloat16
LANES = 128
SUB = 8


def _tree_sum(xs):
    xs = list(xs)
    while len(xs) > 1:
        xs = [xs[i] + xs[i + 1] if i + 1 < len(xs) else xs[i] for i in range(0, len(xs), 2)]
    return xs[0]


def _layernorm(x, eps=1e-5):
    m = jnp.mean(x, axis=-1, keepdims=True)
    d = x - m
    v = jnp.mean(d * d, axis=-1, keepdims=True)
    return d / jnp.sqrt(v + eps)


def _spread(i, n, a):
    return (i & (a - 1)) * (n // a) + (i >> (a.bit_length() - 1))


def _make(L0=16, L1=24, S=32, d=0, dm=None, dq=None, dk=None, dv=None, do=None, d1=None, d2=None,
         am=4, aq=8, ao=8, a1=2, a2=2, kv='half', nobc=True, nosc=True, start_delay=0, compute=True):
    LAG = (L0, L1)
    assert S & (S - 1) == 0
    dm, dq, dk, dv, do, d1, d2 = (d if v is None else v for v in (dm, dq, dk, dv, do, d1, d2))

    def fn(A_x, A_k_cache, A_v_cache, A_wq, A_wo, B_x, B_w1, B_b1, B_w2, c, w_mod):
        del B_x
        D = A_x.shape[-1]
        _, H, SK, DH = A_k_cache.shape
        W = min(4096, max(256, SK // 4))
        F = B_w1.shape[1]
        NM = w_mod.shape[1]
        HD = H * DH
        MB = NM // 2
        QB = 2048
        WB = W // 2
        n_d = D // (2 * SUB)
        n_mb = NM // MB
        n_qb = HD // QB
        n_kv = DH // SUB
        RO = 24
        n_o = HD // (2 * RO)
        n_f2 = F // (2 * RO)
        base_q = n_mb * n_d
        base_h = base_q + n_qb * n_d
        base_o = base_h + 2 * n_kv * H
        base_f1 = base_o + n_o
        base_f2 = base_f1 + n_d
        assert max(LAG) <= min(n_kv, S)
        scale = float(DH) ** -0.5

        def kernel(x_hbm, k_hbm, v_hbm, wq_hbm, wo_hbm, w1_hbm, b1_hbm, w2_hbm, c_hbm, wm_hbm,
                   o_ref,
                   wm_v, wq_v, k_v, v_v, wo_v, w1_v, w2_v, x_v, c_v, b1_v,
                   mod_v, col_v, q_v, s_v, ob_v, sems, small_sems):

            def sem(t, step):
                return sems.at[t, step & (S - 1)]

            def cp_wide(src, dst, base, width, a, t, blk, i):
                c0 = blk * width
                if not isinstance(c0, int):
                    c0 = pl.multiple_of(c0, LANES)
                return pltpu.make_async_copy(src.at[t, _spread(i, n_d, a), :, pl.ds(c0, width)],
                                             dst.at[blk, i, t], sem(t, base + blk * n_d + i))

            cp_m = functools.partial(cp_wide, wm_hbm, wm_v, 0, MB, am)
            cp_q = functools.partial(cp_wide, wq_hbm, wq_v, base_q, QB, aq)

            def kv_pos(t, i):
                if kv == 'half':
                    return t * (n_kv // 2) + (i >> 1), i & 1
                if kv == 'alt':
                    return 2 * (i >> 1) + t, i & 1
                half = (i >= n_kv // 2) * 1
                r = i - half * (n_kv // 2)
                if kv == 'half_r':
                    return t * (n_kv // 2) + r, half
                if kv == 'alt_r':
                    return 2 * r + t, half

            def cp_kv(src, dst, which, h, t, i):
                g, half = kv_pos(t, i)
                c0 = SK - W + half * WB
                if not isinstance(c0, int):
                    c0 = pl.multiple_of(c0, WB)
                return pltpu.make_async_copy(src.at[h * n_kv + g, :, pl.ds(c0, WB)], dst.at[i, t],
                                             sem(t, base_h + (2 * h + which) * n_kv + i))

            cp_k = functools.partial(cp_kv, k_hbm, k_v, 0)
            cp_v = functools.partial(cp_kv, v_hbm, v_v, 1)

            def cp_rows(src, dst, base, n, a, t, i):
                return pltpu.make_async_copy(src.at[t, _spread(i, n, a)], dst.at[i, t], sem(t, base + i))

            cp_o = functools.partial(cp_rows, wo_hbm, wo_v, base_o, n_o, ao)
            cp_f1 = functools.partial(cp_rows, w1_hbm, w1_v, base_f1, n_d, a1)
            cp_f2 = functools.partial(cp_rows, w2_hbm, w2_v, base_f2, n_f2, a2)

            def start(cp, *args):
                return lambda t, *i: cp(*args, t, *i).start(priority=t)

            def advance(wait, start_ahead, pace):
                for t in (0, 1):
                    wait(t)
                for t in (0, 1):
                    start_ahead(t)
                if pace:
                    pl.delay(pace)

            def flat(n, cp, start_next, pace):
                def step(i):
                    def start_ahead(t):
                        nxt = i + LAG[t]
                        pl.when(nxt < n)(lambda: start(cp)(t, nxt))
                        if start_next is not None:
                            pl.when(nxt >= n)(lambda: start_next(t, nxt - n))
                    advance(lambda t: cp(t, i).wait(), start_ahead, pace)
                return step

            def blocked(n_blk, cp, start_next, pace):
                def step(blk, i):
                    def start_ahead(t):
                        nxt = i + LAG[t]
                        wrap = (nxt >= n_d).astype(jnp.int32)
                        nblk, ni = blk + wrap, nxt - wrap * n_d
                        pl.when(nblk < n_blk)(lambda: start(cp)(t, nblk, ni))
                        pl.when(nblk == n_blk)(lambda: start_next(t, ni))
                    advance(lambda t: cp(t, blk, i).wait(), start_ahead, pace)
                return step

            def put_cols(v):
                for j in range(v.shape[1] // LANES):
                    t = jnp.broadcast_to(v[:, j * LANES:(j + 1) * LANES], (LANES, LANES)).T
                    for g in range(LANES // SUB):
                        col_v[j * (LANES // SUB) + g] = t[g * SUB:(g + 1) * SUB]

            def scaled(w, col):
                w = w.astype(F32)
                return w * jnp.tile(col, (1, w.shape[1] // LANES))

            def matvec(n, step, tiles, width):
                def body(i, acc):
                    step(i)
                    if not compute:
                        return acc
                    return acc + _tree_sum(scaled(w, col) for w, col in tiles(i))
                acc = lax.fori_loop(0, n, body, jnp.zeros((SUB, width), F32))
                return jnp.sum(acc, axis=0, keepdims=True)

            def wide_tiles(ref, a):
                return lambda i: [(ref[i, t], col_v[t * n_d + _spread(i, n_d, a)]) for t in (0, 1)]

            cp_c = pltpu.make_async_copy(c_hbm, c_v, small_sems.at[0])
            cp_x = pltpu.make_async_copy(x_hbm, x_v, small_sems.at[1])
            cp_b = pltpu.make_async_copy(b1_hbm, b1_v, small_sems.at[2])
            cp_c.start()
            for i in range(max(LAG)):
                for t in (0, 1):
                    if i < LAG[t]:
                        start(cp_m)(t, 0, i)
                if start_delay and i < LAG[0]:
                    pl.delay(start_delay)
            cp_x.start()
            cp_b.start()

            cp_c.wait()
            cf = c_v[...].astype(F32)
            put_cols(cf * jax.nn.sigmoid(cf))
            step_m = blocked(n_mb, cp_m, lambda t, i: start(cp_q)(t, 0, i), dm)

            def m_block(blk, _):
                mod_v[blk] = matvec(n_d, functools.partial(step_m, blk), wide_tiles(wm_v.at[blk], am), MB)
            lax.fori_loop(0, n_mb, m_block, None)
            sa, ca, ga = (mod_v[0, :, j * D:(j + 1) * D] for j in range(3))
            sb, cb_, gb = (mod_v[1, :, j * D:(j + 1) * D] for j in range(3))
            cp_x.wait()
            x = x_v[0].astype(F32)
            put_cols(_layernorm(x) * (1.0 + ca) + sa)

            step_q = blocked(n_qb, cp_q, start(cp_k, 0), dq)

            def q_block(blk, _):
                q = matvec(n_d, functools.partial(step_q, blk), wide_tiles(wq_v.at[blk], aq), QB) * scale
                for j in range(QB // LANES):
                    q_v[blk * (QB // LANES) + j] = jnp.broadcast_to(q[:, j * LANES:(j + 1) * LANES], (SUB, LANES))
            lax.fori_loop(0, n_qb, q_block, None)

            diag = (lax.broadcasted_iota(jnp.int32, (SUB, LANES), 1)
                    - lax.broadcasted_iota(jnp.int32, (SUB, LANES), 0))

            def lane_sum(v):
                return jnp.broadcast_to(jnp.sum(v, axis=1, keepdims=True), (SUB, LANES))

            def lane_tiles(v):
                return [v[:, j * LANES:(j + 1) * LANES] for j in range(v.shape[1] // LANES)]

            def q_cols(h):
                for i in range(n_kv):
                    g = h * n_kv + i
                    col_v[i] = lane_sum(jnp.where(diag == (g & 15) * SUB, q_v[g >> 4], 0.0))

            q_cols(0)

            def head(h, _):
                s_v[...] = jnp.zeros(s_v.shape, F32)
                step_k = flat(n_kv, functools.partial(cp_k, h), start(cp_v, h), dk)

                def qk(i, _):
                    step_k(i)
                    if compute:
                        half = kv_pos(0, i)[1]
                        s_v[half] += _tree_sum(scaled(k_v[i, t], col_v[kv_pos(t, i)[0]]) for t in (0, 1))
                lax.fori_loop(0, n_kv, qk, None)

                s = [jnp.sum(s_v[j], axis=0, keepdims=True) for j in (0, 1)]
                m = jnp.max(jnp.maximum(s[0], s[1]), axis=1, keepdims=True)
                e = [jnp.exp(sj - m) for sj in s]
                for j in (0, 1):
                    s_v[j] = jnp.broadcast_to(e[j], (SUB, WB))
                denom = _tree_sum(lane_tiles(e[0] + e[1]))

                def start_next(t, i):
                    pl.when(h + 1 < H)(lambda: start(cp_k, h + 1)(t, i))
                    pl.when(h + 1 == H)(lambda: start(cp_o)(t, i))

                step_v = flat(n_kv, functools.partial(cp_v, h), start_next, dv)

                def pv(i, _):
                    step_v(i)
                    if compute:
                        for t in (0, 1):
                            g, half = kv_pos(t, i)
                            col_v[(1 + half) * n_kv + g] = _tree_sum(lane_tiles(v_v[i, t].astype(F32) * s_v[half]))
                lax.fori_loop(0, n_kv, pv, None)

                inv = 1.0 / lane_sum(jnp.broadcast_to(denom, (SUB, LANES)))
                for g in range(n_kv):
                    ob_v[h * n_kv + g] = lane_sum(col_v[n_kv + g] + col_v[2 * n_kv + g]) * inv
                q_cols(jnp.minimum(h + 1, H - 1))
            lax.fori_loop(0, H, head, None)

            per = RO // SUB

            def tall_tiles(ref, cols, n, a):
                return lambda i: [(ref[i, t, pl.ds(r * SUB, SUB), :], cols[(t * n + _spread(i, n, a)) * per + r])
                                  for t in (0, 1) for r in range(per)]
            attn = matvec(n_o, flat(n_o, cp_o, start(cp_f1), do), tall_tiles(wo_v, ob_v, n_o, ao), D)
            x1 = x + ga * attn
            put_cols(_layernorm(x1) * (1.0 + cb_) + sb)

            a = matvec(n_d, flat(n_d, cp_f1, start(cp_f2), d1), wide_tiles(w1_v, a1), F)
            cp_b.wait()
            a = a + b1_v[...].astype(F32).reshape(1, F)
            sp = jnp.log1p(jnp.exp(-jnp.abs(a))) + jnp.where(a > 0, a, 0.0)
            put_cols(a * jnp.tanh(sp))
            y = matvec(n_f2, flat(n_f2, cp_f2, None, d2), tall_tiles(w2_v, col_v, n_f2, a2), D)
            o_ref[0] = (x1 + gb * y).astype(o_ref.dtype)

        any_spec = pl.BlockSpec(memory_space=pl.ANY)
        kt = jnp.swapaxes(A_k_cache, 2, 3).reshape(H * n_kv, SUB, SK)
        vt = jnp.swapaxes(A_v_cache, 2, 3).reshape(H * n_kv, SUB, SK)
        return pl.pallas_call(
            kernel,
            out_shape=jax.ShapeDtypeStruct(A_x.shape, A_x.dtype),
            in_specs=[any_spec] * 10,
            out_specs=pl.BlockSpec(memory_space=pltpu.VMEM),
            scratch_shapes=[
                pltpu.VMEM((n_mb, n_d, 2, SUB, MB), BF16),
                pltpu.VMEM((n_qb, n_d, 2, SUB, QB), BF16),
                pltpu.VMEM((n_kv, 2, SUB, WB), BF16),
                pltpu.VMEM((n_kv, 2, SUB, WB), BF16),
                pltpu.VMEM((n_o, 2, RO, D), BF16),
                pltpu.VMEM((n_d, 2, SUB, F), BF16),
                pltpu.VMEM((n_f2, 2, RO, D), BF16),
                pltpu.VMEM(A_x.shape, BF16),
                pltpu.VMEM(c.shape, BF16),
                pltpu.VMEM(B_b1.shape, BF16),
                pltpu.VMEM((n_mb, 1, MB), F32),
                pltpu.VMEM((F // SUB, SUB, LANES), F32),
                pltpu.VMEM((HD // LANES, SUB, LANES), F32),
                pltpu.VMEM((2, SUB, WB), F32),
                pltpu.VMEM((HD // SUB, SUB, LANES), F32),
                pltpu.SemaphoreType.DMA((2, S)),
                pltpu.SemaphoreType.DMA((3,)),
            ],
            compiler_params=pltpu.CompilerParams(vmem_limit_bytes=64 * 1024 * 1024, disable_bounds_checks=nobc,
                                                 disable_semaphore_checks=nosc),
        )(A_x, kt, vt, A_wq.reshape(2, n_d, SUB, HD), A_wo.reshape(2, n_o, RO, D),
          B_w1.reshape(2, n_d, SUB, F), B_b1, B_w2.reshape(2, n_f2, RO, D), c,
          w_mod.reshape(2, n_d, SUB, NM))

    return fn


@jax.jit
def pallas_adaLN_cond__sliding_block_cached__dense_activation_mish__decode_kernel(
    A_x: jax.Array,
    A_k_cache: jax.Array,
    A_v_cache: jax.Array,
    A_wq: jax.Array,
    A_wo: jax.Array,
    B_x: jax.Array,
    B_w1: jax.Array,
    B_b1: jax.Array,
    B_w2: jax.Array,
    c: jax.Array,
    w_mod: jax.Array,
):
    return _make()(A_x, A_k_cache, A_v_cache, A_wq, A_wo, B_x, B_w1, B_b1, B_w2, c, w_mod)
```

```python
import functools

import jax
import jax.numpy as jnp
from jax import lax
from jax.experimental import pallas as pl
from jax.experimental.pallas import tpu as pltpu

F32 = jnp.float32
BF16 = jnp.bfloat16
LANES = 128
SUB = 8
P = 4


def _tree_sum(xs):
    xs = list(xs)
    while len(xs) > 1:
        xs = [xs[i] + xs[i + 1] if i + 1 < len(xs) else xs[i] for i in range(0, len(xs), 2)]
    return xs[0]


def _layernorm(x, eps=1e-5):
    m = jnp.mean(x, axis=-1, keepdims=True)
    d = x - m
    v = jnp.mean(d * d, axis=-1, keepdims=True)
    return d / jnp.sqrt(v + eps)


def _slabs(w, tiles, lead):
    r, c = w.shape
    w = w.reshape(r // SUB, SUB, c // LANES, LANES).transpose(0, 2, 1, 3)
    return w.reshape(*lead, -1, SUB * tiles, LANES)


def _make(L0=12, L1=16, S=32, d=0, dm=None, dq=None, dk=None, dv=None, do=None, d1=None, d2=None,
         nobc=True, nosc=True, start_delay=0, compute=True, sk=0):
    LAG = (L0, L1)
    assert S & (S - 1) == 0
    dm, dq, dk, dv, do, d1, d2 = (d if v is None else v for v in (dm, dq, dk, dv, do, d1, d2))

    def fn(A_x, A_k_cache, A_v_cache, A_wq, A_wo, B_x, B_w1, B_b1, B_w2, c, w_mod):
        del B_x
        D = A_x.shape[-1]
        _, H, SK, DH = A_k_cache.shape
        W = min(4096, max(256, SK // 4))
        F = B_w1.shape[1]
        NM = w_mod.shape[1]
        HD = H * DH
        TC, TD = 4, D // LANES
        CB = TC * LANES
        RS = 2 * P * SUB
        n_d = D // RS
        n_h = DH // RS
        n_o = HD // RS
        n_f = F // RS
        b_m, b_q, b_w, b_f = NM // D, HD // CB, W // CB, F // CB
        g_h = DH // SUB
        n_kv = b_w * n_h
        base_q = b_m * n_d
        base_h = base_q + b_q * n_d
        base_o = base_h + 2 * n_kv * H
        base_f1 = base_o + n_o
        base_f2 = base_f1 + b_f * n_d
        assert max(LAG) <= min(n_kv, n_f, S)
        scale = float(DH) ** -0.5

        def kernel(x_hbm, k_hbm, v_hbm, wq_hbm, wo_hbm, w1_hbm, b1_hbm, w2_hbm, c_hbm, wm_hbm,
                   o_ref,
                   wm_v, wq_v, k_v, v_v, wo_v, w1_v, w2_v, x_v, c_v, b1_v,
                   acc_v, col_v, q_v, s_v, ob_v, sems, small_sems):

            def sem(t, step):
                return sems.at[t, step & (S - 1)]

            def cp_w(src, dst, base, t, i):
                return pltpu.make_async_copy(src.at[t, :, i], dst.at[i, t], sem(t, base + i))

            cp_m = functools.partial(cp_w, wm_hbm, wm_v, 0)
            cp_q = functools.partial(cp_w, wq_hbm, wq_v, base_q)
            cp_o = functools.partial(cp_w, wo_hbm, wo_v, base_o)
            cp_f1 = functools.partial(cp_w, w1_hbm, w1_v, base_f1)
            cp_f2 = functools.partial(cp_w, w2_hbm, w2_v, base_f2)

            def cp_kv(src, dst, which, h, t, blk, r):
                return pltpu.make_async_copy(src.at[h, t, r, :, (SK - W) // CB - sk + blk], dst.at[blk, r, t],
                                             sem(t, base_h + (2 * h + which) * n_kv + blk * n_h + r))

            cp_k = functools.partial(cp_kv, k_hbm, k_v, 0)
            cp_v = functools.partial(cp_kv, v_hbm, v_v, 1)

            def run_step(wait, work, refill, pace):
                for t in (0, 1):
                    wait(t)
                out = work() if compute else None
                for t in (0, 1):
                    refill(t)
                if pace:
                    pl.delay(pace)
                return out

            def w_step(n, cp, cp_next, pace, i, work):
                def refill(t):
                    nxt = i + LAG[t]
                    pl.when(nxt < n)(lambda: cp(t, nxt).start(priority=t))
                    if cp_next is not None:
                        pl.when(nxt >= n)(lambda: cp_next(t, nxt - n).start(priority=t))
                return run_step(lambda t: cp(t, i).wait(), work, refill, pace)

            def kv_step(cp, start_next, pace, blk, r, work):
                def refill(t):
                    ahead, nr = divmod(r + LAG[t], n_h)
                    nblk = blk + ahead
                    pl.when(nblk < b_w)(lambda: cp(t, nblk, nr).start(priority=t))
                    start_next(t, nblk >= b_w, nblk - b_w, nr)
                return run_step(lambda t: cp(t, blk, r).wait(), work, refill, pace)

            def tiles(w):
                w = w.astype(F32)
                return [w[j * SUB:(j + 1) * SUB] for j in range(w.shape[0] // SUB)]

            def put_cols(v):
                for j in range(v.shape[1] // LANES):
                    t = jnp.broadcast_to(v[:, j * LANES:(j + 1) * LANES], (LANES, LANES)).T
                    for g in range(LANES // SUB):
                        col_v[j * (LANES // SUB) + g] = t[g * SUB:(g + 1) * SUB]

            def partial_dot(ref, cols):
                prods = [[w * cols[t * P + p] for w in tiles(ref[t, p])] for t in (0, 1) for p in range(P)]
                return [_tree_sum(col) for col in zip(*prods)]

            def row_of(parts):
                return jnp.concatenate([jnp.sum(p, axis=0, keepdims=True) for p in parts], axis=1)

            def wide(n_blk, ref, cp, cp_next, pace):
                nt = ref.shape[-2] // SUB
                for j in range(n_blk * nt):
                    acc_v[j] = jnp.zeros((SUB, LANES), F32)

                def rows(r, _):
                    cols = [col_v[j * n_d + r] for j in range(2 * P)]

                    def block(blk, _):
                        i = r * n_blk + blk

                        def work():
                            for j, part in enumerate(partial_dot(ref.at[i], cols)):
                                acc_v[blk * nt + j] += part
                        w_step(n_blk * n_d, cp, cp_next, pace, i, work)
                    lax.fori_loop(0, n_blk, block, None)
                lax.fori_loop(0, n_d, rows, None)

            def tall(n, ref, col_ref, cp, cp_next, pace):
                def body(i, acc):
                    def work():
                        cols = [col_ref[j * n + i] for j in range(2 * P)]
                        return [a + part for a, part in zip(acc, partial_dot(ref.at[i], cols))]
                    return w_step(n, cp, cp_next, pace, i, work) or acc
                return row_of(lax.fori_loop(0, n, body, [jnp.zeros((SUB, LANES), F32)] * TD))

            cp_c = pltpu.make_async_copy(c_hbm, c_v, small_sems.at[0])
            cp_x = pltpu.make_async_copy(x_hbm, x_v, small_sems.at[1])
            cp_b = pltpu.make_async_copy(b1_hbm, b1_v, small_sems.at[2])
            cp_c.start()
            for i in range(max(LAG)):
                for t in (0, 1):
                    if i < LAG[t]:
                        cp_m(t, i).start(priority=t)
                if start_delay and i < LAG[0]:
                    pl.delay(start_delay)
            cp_x.start()
            cp_b.start()

            cp_c.wait()
            cf = c_v[...].astype(F32)
            put_cols(cf * jax.nn.sigmoid(cf))
            wide(b_m, wm_v, cp_m, cp_q, dm)
            sa, ca, ga, sb, cb_, gb = (row_of([acc_v[b * TD + j] for j in range(TD)]) for b in range(6))
            cp_x.wait()
            x = x_v[0].astype(F32)
            put_cols(_layernorm(x) * (1.0 + ca) + sa)

            def first_keys(t, i):
                blk = (i * 43) >> 7
                return cp_k(0, t, blk, i - blk * n_h)
            wide(b_q, wq_v, cp_q, first_keys, dq)
            for j in range(HD // LANES):
                q_v[j] = jnp.broadcast_to(jnp.sum(acc_v[j], axis=0, keepdims=True) * scale, (SUB, LANES))

            diag = (lax.broadcasted_iota(jnp.int32, (SUB, LANES), 1)
                    - lax.broadcasted_iota(jnp.int32, (SUB, LANES), 0))

            def lane_sum(v):
                return jnp.broadcast_to(jnp.sum(v, axis=1, keepdims=True), (SUB, LANES))

            def q_cols(h):
                for i in range(g_h):
                    g = h * g_h + i
                    col_v[i] = lane_sum(jnp.where(diag == (g & 15) * SUB, q_v[g >> 4], 0.0))

            def group(t, r, p):
                return (t * n_h + r) * P + p

            q_cols(0)

            def head(h, _):
                def after_k(t, over, blk, r):
                    pl.when(over)(lambda: cp_v(h, t, blk, r).start(priority=t))

                def k_block(blk, top):
                    acc = None
                    for r in range(n_h):
                        def work():
                            cols = [col_v[group(t, r, p)] for t in (0, 1) for p in range(P)]
                            return partial_dot(k_v.at[blk, r], cols)
                        part = kv_step(functools.partial(cp_k, h), after_k, dk, blk, r, work)
                        acc = part if acc is None else [a + b for a, b in zip(acc, part)]
                    if not compute:
                        return top
                    for j in range(TC):
                        s = jnp.broadcast_to(jnp.sum(acc[j], axis=0, keepdims=True), (SUB, LANES))
                        s_v[blk, j] = s
                        top = jnp.maximum(top, s)
                    return top
                top = lax.fori_loop(0, b_w, k_block, jnp.full((SUB, LANES), -jnp.inf, F32))
                top = jnp.max(top, axis=1, keepdims=True)
                for g in range(g_h):
                    acc_v[g] = jnp.zeros((SUB, LANES), F32)

                def after_v(t, over, blk, r):
                    pl.when(over & (h + 1 < H))(lambda: cp_k(h + 1, t, blk, r).start(priority=t))
                    pl.when(over & (h + 1 == H))(lambda: cp_o(t, blk * n_h + r).start(priority=t))

                def v_block(blk, denom):
                    e = [jnp.exp(s_v[blk, j] - top) for j in range(TC)]
                    for r in range(n_h):
                        def work():
                            for t in (0, 1):
                                for p in range(P):
                                    acc_v[group(t, r, p)] += _tree_sum(
                                        w * ej for w, ej in zip(tiles(v_v[blk, r, t, p]), e))
                        kv_step(functools.partial(cp_v, h), after_v, dv, blk, r, work)
                    return denom + _tree_sum(e)
                denom = lax.fori_loop(0, b_w, v_block, jnp.zeros((SUB, LANES), F32))

                inv = 1.0 / lane_sum(denom)
                for g in range(g_h):
                    ob_v[h * g_h + g] = lane_sum(acc_v[g]) * inv
                q_cols(jnp.minimum(h + 1, H - 1))
            lax.fori_loop(0, H, head, None)

            x1 = x + ga * tall(n_o, wo_v, ob_v, cp_o, cp_f1, do)
            put_cols(_layernorm(x1) * (1.0 + cb_) + sb)

            wide(b_f, w1_v, cp_f1, cp_f2, d1)
            cp_b.wait()
            a = row_of([acc_v[j] for j in range(F // LANES)]) + b1_v[...].astype(F32).reshape(1, F)
            sp = jnp.log1p(jnp.exp(-jnp.abs(a))) + jnp.where(a > 0, a, 0.0)
            put_cols(a * jnp.tanh(sp))
            y = tall(n_f, w2_v, col_v, cp_f2, None, d2)
            o_ref[0] = (x1 + gb * y).astype(o_ref.dtype)

        any_spec = pl.BlockSpec(memory_space=pl.ANY)
        kt = _slabs(jnp.swapaxes(A_k_cache, 2, 3).reshape(HD, SK), TC, (H, 2, n_h, P))
        vt = _slabs(jnp.swapaxes(A_v_cache, 2, 3).reshape(HD, SK), TC, (H, 2, n_h, P))
        return pl.pallas_call(
            kernel,
            out_shape=jax.ShapeDtypeStruct(A_x.shape, A_x.dtype),
            in_specs=[any_spec] * 10,
            out_specs=pl.BlockSpec(memory_space=pltpu.VMEM),
            scratch_shapes=[
                pltpu.VMEM((b_m * n_d, 2, P, SUB * TD, LANES), BF16),
                pltpu.VMEM((b_q * n_d, 2, P, SUB * TC, LANES), BF16),
                pltpu.VMEM((b_w, n_h, 2, P, SUB * TC, LANES), BF16),
                pltpu.VMEM((b_w, n_h, 2, P, SUB * TC, LANES), BF16),
                pltpu.VMEM((n_o, 2, P, SUB * TD, LANES), BF16),
                pltpu.VMEM((b_f * n_d, 2, P, SUB * TC, LANES), BF16),
                pltpu.VMEM((n_f, 2, P, SUB * TD, LANES), BF16),
                pltpu.VMEM(A_x.shape, BF16),
                pltpu.VMEM(c.shape, BF16),
                pltpu.VMEM(B_b1.shape, BF16),
                pltpu.VMEM((HD // LANES, SUB, LANES), F32),
                pltpu.VMEM((F // SUB, SUB, LANES), F32),
                pltpu.VMEM((HD // LANES, SUB, LANES), F32),
                pltpu.VMEM((b_w, TC, SUB, LANES), F32),
                pltpu.VMEM((HD // SUB, SUB, LANES), F32),
                pltpu.SemaphoreType.DMA((2, S)),
                pltpu.SemaphoreType.DMA((3,)),
            ],
            compiler_params=pltpu.CompilerParams(vmem_limit_bytes=64 * 1024 * 1024, disable_bounds_checks=nobc,
                                                 disable_semaphore_checks=nosc),
        )(A_x, kt, vt, _slabs(A_wq, TC, (2, P)), _slabs(A_wo, TD, (2, P)), _slabs(B_w1, TC, (2, P)), B_b1,
          _slabs(B_w2, TD, (2, P)), c, _slabs(w_mod, TD, (2, P)))

    return fn


@jax.jit
def pallas_adaLN_cond__sliding_block_cached__dense_activation_mish__decode_kernel(
    A_x: jax.Array,
    A_k_cache: jax.Array,
    A_v_cache: jax.Array,
    A_wq: jax.Array,
    A_wo: jax.Array,
    B_x: jax.Array,
    B_w1: jax.Array,
    B_b1: jax.Array,
    B_w2: jax.Array,
    c: jax.Array,
    w_mod: jax.Array,
):
    return _make(L0=12,L1=20,d=25,dm=45,do=45,d2=45)(A_x, A_k_cache, A_v_cache, A_wq, A_wo, B_x, B_w1, B_b1, B_w2, c, w_mod)
```

```python
import functools

import jax
import jax.numpy as jnp
from jax import lax
from jax.experimental import pallas as pl
from jax.experimental.pallas import tpu as pltpu

F32 = jnp.float32
BF16 = jnp.bfloat16
LANES = 128
SUB = 8
P = 4


def _tree_sum(xs):
    xs = list(xs)
    while len(xs) > 1:
        xs = [xs[i] + xs[i + 1] if i + 1 < len(xs) else xs[i] for i in range(0, len(xs), 2)]
    return xs[0]


def _layernorm(x, eps=1e-5):
    m = jnp.mean(x, axis=-1, keepdims=True)
    d = x - m
    v = jnp.mean(d * d, axis=-1, keepdims=True)
    return d / jnp.sqrt(v + eps)


def _slabs(w, tiles, lead):
    r, c = w.shape
    w = w.reshape(r // SUB, SUB, c // LANES, LANES).transpose(0, 2, 1, 3)
    return w.reshape(*lead, -1, SUB * tiles, LANES)


def _dispatch(pos, lo, hi, segments):
    start = 0
    for length, go in segments:
        end = start + length
        if start < hi and end > lo:
            conds = ([pos >= start] if start > lo else []) + ([pos < end] if end < hi else [])
            if conds:
                pl.when(functools.reduce(jnp.logical_and, conds))(functools.partial(go, pos - start))
            else:
                go(pos - start)
        start = end


def _make(L0=12, L1=36, S=64, sk=0, scopes=False, PO=4, half=False):
    import contextlib
    scope = jax.named_scope if scopes else (lambda n: contextlib.nullcontext())
    LAG = (L0, L1)

    def fn(A_x, A_k_cache, A_v_cache, A_wq, A_wo, B_x, B_w1, B_b1, B_w2, c, w_mod):
        del B_x
        D = A_x.shape[-1]
        _, H, SK, DH = A_k_cache.shape
        W = min(4096, max(256, SK // 4))
        F = B_w1.shape[1]
        NM = w_mod.shape[1]
        HD = H * DH
        TC, TD = 4, D // LANES
        CB = TC * LANES
        RS = 2 * P * SUB
        n_d = D // RS
        n_h = DH // RS
        n_o = HD // (2 * PO * SUB)
        n_f2 = F // (2 * PO * SUB)
        b_m, b_q, b_w, b_f = NM // D, HD // CB, W // CB, F // CB
        n_m, n_q, n_f1 = b_m * n_d, b_q * n_d, b_f * n_d
        g_h = DH // SUB
        n_kv = b_w * n_h
        base_q = n_m
        base_h = base_q + n_q
        base_o = base_h + 2 * n_kv * H
        base_f1 = base_o + n_o
        base_f2 = base_f1 + n_f1
        assert max(LAG) < min(2 * n_kv, n_m, S)
        scale = float(DH) ** -0.5

        def kernel(x_hbm, k_hbm, v_hbm, wq_hbm, wo_hbm, w1_hbm, b1_hbm, w2_hbm, c_hbm, wm_hbm,
                   o_ref,
                   wm_v, wq_v, k_v, v_v, wo_v, w1_v, w2_v, x_v, c_v, b1_v,
                   acc_v, col_v, q_v, s_v, ob_v, sems, small_sems):

            def sem(t, step):
                return sems.at[t, step & (S - 1)]

            def cp_w(src, dst, base, t, i):
                return pltpu.make_async_copy(src.at[t, :, i], dst.at[i, t], sem(t, base + i))

            cp_m = functools.partial(cp_w, wm_hbm, wm_v, 0)
            cp_q = functools.partial(cp_w, wq_hbm, wq_v, base_q)
            cp_o = functools.partial(cp_w, wo_hbm, wo_v, base_o)
            cp_f1 = functools.partial(cp_w, w1_hbm, w1_v, base_f1)
            cp_f2 = functools.partial(cp_w, w2_hbm, w2_v, base_f2)

            def cp_kv(src, dst, which, h, r, t, blk):
                return pltpu.make_async_copy(src.at[h, t, r, :, (SK - W) // CB - sk + blk], dst.at[blk, r, t],
                                             sem(t, base_h + (2 * h + which) * n_kv + blk * n_h + r))

            cp_k = functools.partial(cp_kv, k_hbm, k_v, 0)
            cp_v = functools.partial(cp_kv, v_hbm, v_v, 1)

            def start(cp, t):
                return lambda i: cp(t, i).start(priority=t)

            def step(wait, work, refill):
                if half:
                    for t in (0, 1):
                        wait(t)
                        work(t)
                        refill(t)
                else:
                    for f in (wait, work, refill):
                        for t in (0, 1):
                            f(t)

            def w_step(streams, i, work):
                n, cp = streams[0]
                step(lambda t: cp(t, i).wait(), work,
                     lambda t: _dispatch(i + LAG[t], LAG[t], LAG[t] + n, [(m, start(c, t)) for m, c in streams]))

            def tiles(w):
                w = w.astype(F32)
                return [w[j * SUB:(j + 1) * SUB] for j in range(w.shape[0] // SUB)]

            def put_cols(v):
                for j in range(v.shape[1] // LANES):
                    t = jnp.broadcast_to(v[:, j * LANES:(j + 1) * LANES], (LANES, LANES)).T
                    for g in range(LANES // SUB):
                        col_v[j * (LANES // SUB) + g] = t[g * SUB:(g + 1) * SUB]

            def partial_dot(ref, cols):
                prods = [[w * col for w in tiles(ref[p])] for p, col in enumerate(cols)]
                return [_tree_sum(col) for col in zip(*prods)]

            def row_of(parts):
                return jnp.concatenate([jnp.sum(p, axis=0, keepdims=True) for p in parts], axis=1)

            def wide(v, ref, streams):
                nt = ref.shape[-2] // SUB
                n_blk = streams[0][0] // n_d
                put_cols(v)
                for j in range(n_blk * nt):
                    acc_v[j] = jnp.zeros((SUB, LANES), F32)

                def rows(r, _):
                    cols = [col_v[j * n_d + r] for j in range(2 * P)]

                    def block(blk, _):
                        i = r * n_blk + blk
                        parts = [[acc_v[blk * nt + j] for j in range(nt)]]
                        w_step(streams, i,
                               lambda t: parts.append(partial_dot(ref.at[i, t], cols[t * P:(t + 1) * P])))
                        for j, col in enumerate(zip(*parts)):
                            acc_v[blk * nt + j] = _tree_sum(col[::-1])
                    lax.fori_loop(0, n_blk, block, None)
                lax.fori_loop(0, n_d, rows, None)

            def tall(col_ref, ref, streams):
                n = streams[0][0]

                def body(i, acc):
                    parts = [acc]
                    w_step(streams, i, lambda t: parts.append(
                        partial_dot(ref.at[i, t], [col_ref[(t * PO + p) * n + i] for p in range(PO)])))
                    return [_tree_sum(col[::-1]) for col in zip(*parts)]
                return row_of(lax.fori_loop(0, n, body, [jnp.zeros((SUB, LANES), F32)] * TD))

            cp_c = pltpu.make_async_copy(c_hbm, c_v, small_sems.at[0])
            cp_x = pltpu.make_async_copy(x_hbm, x_v, small_sems.at[1])
            cp_b = pltpu.make_async_copy(b1_hbm, b1_v, small_sems.at[2])
            cp_c.start()
            cp_x.start()
            cp_b.start()

            def prime(i, _):
                for t in (0, 1):
                    _dispatch(i, 0, max(LAG), [(LAG[t], start(cp_m, t))])
            lax.fori_loop(0, max(LAG), prime, None)

            cp_c.wait()
            cf = c_v[...].astype(F32)
            with scope('ph_M'):
                wide(cf * jax.nn.sigmoid(cf), wm_v, [(n_m, cp_m), (n_q, cp_q)])
            sa, ca, ga, sb, cb_, gb = (row_of([acc_v[b * TD + j] for j in range(TD)]) for b in range(6))
            cp_x.wait()
            x = x_v[0].astype(F32)

            def first_head(cp):
                def flat(t, i):
                    blk = (i * 43) >> 7
                    return cp(0, i - blk * n_h, t, blk)
                return flat
            with scope('ph_Q'):
                wide(_layernorm(x) * (1.0 + ca) + sa, wq_v,
                     [(n_q, cp_q), (n_kv, first_head(cp_k)), (n_kv, first_head(cp_v))])
            for j in range(HD // LANES):
                q_v[j] = jnp.broadcast_to(jnp.sum(acc_v[j], axis=0, keepdims=True) * scale, (SUB, LANES))

            diag = (lax.broadcasted_iota(jnp.int32, (SUB, LANES), 1)
                    - lax.broadcasted_iota(jnp.int32, (SUB, LANES), 0))

            def lane_sum(v):
                return jnp.broadcast_to(jnp.sum(v, axis=1, keepdims=True), (SUB, LANES))

            def q_cols(h):
                for i in range(g_h):
                    g = h * g_h + i
                    col_v[i] = lane_sum(jnp.where(diag == (g & 15) * SUB, q_v[g >> 4], 0.0))

            def group(t, r, p):
                return (t * n_h + r) * P + p

            q_cols(0)

            def head(h, _):
                def kv_step(which, blk, r, work):
                    def refill(t):
                        ahead, nr = divmod(r + LAG[t], n_h)
                        ahead += which * b_w

                        def next_head(cp):
                            return lambda b: pl.when(h + 1 < H)(
                                lambda: cp(h + 1, nr, t, b).start(priority=t))

                        def out_proj(b):
                            pl.when(h + 1 == H)(lambda: cp_o(t, b * n_h + nr).start(priority=t))
                        _dispatch(blk + ahead, ahead, ahead + b_w,
                                  [(b_w, start(functools.partial(cp_k, h, nr), t)),
                                   (b_w, start(functools.partial(cp_v, h, nr), t)),
                                   (b_w, next_head(cp_k)), (b_w, next_head(cp_v))])
                        _dispatch(blk + ahead, ahead, ahead + b_w, [(2 * b_w, lambda b: None), (2 * b_w, out_proj)])
                    step(lambda t: (cp_k, cp_v)[which](h, r, t, blk).wait(), work, refill)

                def k_block(blk, top):
                    parts = []
                    for r in range(n_h):
                        kv_step(0, blk, r, lambda t: parts.append(
                            partial_dot(k_v.at[blk, r, t], [col_v[group(t, r, p)] for p in range(P)])))
                        parts[:] = [[_tree_sum(col[::-1]) for col in zip(*parts)]]
                    for j in range(TC):
                        s = jnp.broadcast_to(jnp.sum(parts[0][j], axis=0, keepdims=True), (SUB, LANES))
                        s_v[blk, j] = s
                        top = jnp.maximum(top, s)
                    return top
                top = lax.fori_loop(0, b_w, k_block, jnp.full((SUB, LANES), -jnp.inf, F32))
                top = jnp.max(top, axis=1, keepdims=True)
                for g in range(g_h):
                    acc_v[g] = jnp.zeros((SUB, LANES), F32)

                def v_block(blk, denom):
                    e = [jnp.exp(s_v[blk, j] - top) for j in range(TC)]
                    for r in range(n_h):
                        def work(t):
                            for p in range(P):
                                acc_v[group(t, r, p)] += _tree_sum(
                                    w * ej for w, ej in zip(tiles(v_v[blk, r, t, p]), e))
                        kv_step(1, blk, r, work)
                    return denom + _tree_sum(e)
                denom = lax.fori_loop(0, b_w, v_block, jnp.zeros((SUB, LANES), F32))

                inv = 1.0 / lane_sum(denom)
                for g in range(g_h):
                    ob_v[h * g_h + g] = lane_sum(acc_v[g]) * inv
                q_cols(jnp.minimum(h + 1, H - 1))
            with scope('ph_H'):
                lax.fori_loop(0, H, head, None)

            with scope('ph_O'):
                attn = tall(ob_v, wo_v, [(n_o, cp_o), (n_f1, cp_f1), (n_f2, cp_f2)])
            x1 = x + ga * attn

            with scope('ph_F1'):
                wide(_layernorm(x1) * (1.0 + cb_) + sb, w1_v, [(n_f1, cp_f1), (n_f2, cp_f2)])
            cp_b.wait()
            a = row_of([acc_v[j] for j in range(F // LANES)]) + b1_v[...].astype(F32).reshape(1, F)
            sp = jnp.log1p(jnp.exp(-jnp.abs(a))) + jnp.where(a > 0, a, 0.0)
            put_cols(a * jnp.tanh(sp))
            with scope('ph_F2'):
                y = tall(col_v, w2_v, [(n_f2, cp_f2)])
            o_ref[0] = (x1 + gb * y).astype(o_ref.dtype)

        any_spec = pl.BlockSpec(memory_space=pl.ANY)
        kt = _slabs(jnp.swapaxes(A_k_cache, 2, 3).reshape(HD, SK), TC, (H, 2, n_h, P))
        vt = _slabs(jnp.swapaxes(A_v_cache, 2, 3).reshape(HD, SK), TC, (H, 2, n_h, P))
        return pl.pallas_call(
            kernel,
            out_shape=jax.ShapeDtypeStruct(A_x.shape, A_x.dtype),
            in_specs=[any_spec] * 10,
            out_specs=pl.BlockSpec(memory_space=pltpu.VMEM),
            scratch_shapes=[
                pltpu.VMEM((n_m, 2, P, SUB * TD, LANES), BF16),
                pltpu.VMEM((n_q, 2, P, SUB * TC, LANES), BF16),
                pltpu.VMEM((b_w, n_h, 2, P, SUB * TC, LANES), BF16),
                pltpu.VMEM((b_w, n_h, 2, P, SUB * TC, LANES), BF16),
                pltpu.VMEM((n_o, 2, PO, SUB * TD, LANES), BF16),
                pltpu.VMEM((n_f1, 2, P, SUB * TC, LANES), BF16),
                pltpu.VMEM((n_f2, 2, PO, SUB * TD, LANES), BF16),
                pltpu.VMEM(A_x.shape, BF16),
                pltpu.VMEM(c.shape, BF16),
                pltpu.VMEM(B_b1.shape, BF16),
                pltpu.VMEM((HD // LANES, SUB, LANES), F32),
                pltpu.VMEM((F // SUB, SUB, LANES), F32),
                pltpu.VMEM((HD // LANES, SUB, LANES), F32),
                pltpu.VMEM((b_w, TC, SUB, LANES), F32),
                pltpu.VMEM((HD // SUB, SUB, LANES), F32),
                pltpu.SemaphoreType.DMA((2, S)),
                pltpu.SemaphoreType.DMA((3,)),
            ],
            compiler_params=pltpu.CompilerParams(vmem_limit_bytes=64 * 1024 * 1024, disable_bounds_checks=True,
                                                 disable_semaphore_checks=True),
        )(A_x, kt, vt, _slabs(A_wq, TC, (2, P)), _slabs(A_wo, TD, (2, PO)), _slabs(B_w1, TC, (2, P)), B_b1,
          _slabs(B_w2, TD, (2, PO)), c, _slabs(w_mod, TD, (2, P)))

    return fn


@jax.jit
def pallas_adaLN_cond__sliding_block_cached__dense_activation_mish__decode_kernel(
    A_x: jax.Array,
    A_k_cache: jax.Array,
    A_v_cache: jax.Array,
    A_wq: jax.Array,
    A_wo: jax.Array,
    B_x: jax.Array,
    B_w1: jax.Array,
    B_b1: jax.Array,
    B_w2: jax.Array,
    c: jax.Array,
    w_mod: jax.Array,
):
    return _make()(A_x, A_k_cache, A_v_cache, A_wq, A_wo, B_x, B_w1, B_b1, B_w2, c, w_mod)
```

```python
import functools

import jax
import jax.numpy as jnp
from jax import lax
from jax.experimental import pallas as pl
from jax.experimental.pallas import tpu as pltpu

F32 = jnp.float32
LANES = 128
SUB = 8
QUEUES = (0, 1)
LAG = (12, 36)
RING = 64
RUNS = 4
RUNS_TALL = 3
RUN_TILES = 4
HOPS = 5


def _div(i, d, bound):
    shift = (bound * d).bit_length()
    mul = -(-(1 << shift) // d)
    assert all((j * mul) >> shift == j // d for j in range(bound)) and bound * mul < 2**31
    return (i * mul) >> shift


def _tree_sum(xs):
    xs = list(xs)
    while len(xs) > 1:
        xs = [xs[i] + xs[i + 1] if i + 1 < len(xs) else xs[i] for i in range(0, len(xs), 2)]
    return xs[0]


def _layernorm(x, eps=1e-5):
    d = x - jnp.mean(x, axis=-1, keepdims=True)
    return d / jnp.sqrt(jnp.mean(d * d, axis=-1, keepdims=True) + eps)


def _runs(w, tiles, lead):
    r, c = w.shape
    w = w.reshape(r // SUB, SUB, c // LANES, LANES).transpose(0, 2, 1, 3)
    return w.reshape(*lead, -1, SUB * tiles, LANES)


def _dispatch(pos, lo, hi, segments):
    start = 0
    for length, go in segments:
        end = start + length
        if start < hi and end > lo:
            conds = ([pos >= start] if start > lo else []) + ([pos < end] if end < hi else [])
            if conds:
                pl.when(functools.reduce(jnp.logical_and, conds))(functools.partial(go, pos - start))
            else:
                go(pos - start)
        start = end


@jax.jit
def pallas_adaLN_cond__sliding_block_cached__dense_activation_mish__decode_kernel(
    A_x: jax.Array,
    A_k_cache: jax.Array,
    A_v_cache: jax.Array,
    A_wq: jax.Array,
    A_wo: jax.Array,
    B_x: jax.Array,
    B_w1: jax.Array,
    B_b1: jax.Array,
    B_w2: jax.Array,
    c: jax.Array,
    w_mod: jax.Array,
):
    del B_x
    D = A_x.shape[-1]
    _, H, SK, DH = A_k_cache.shape
    W = min(4096, max(256, SK // 4))
    F = B_w1.shape[1]
    HD = H * DH
    TC, TD = RUN_TILES, D // LANES
    CB = TC * LANES
    rows, rows_tall = 2 * RUNS * SUB, 2 * RUNS_TALL * SUB
    n_d, n_h = D // rows, DH // rows
    b_m, b_q, b_w, b_f = w_mod.shape[1] // D, HD // CB, W // CB, F // CB
    g_h = DH // SUB
    n_m, n_q, n_kv, n_f1 = b_m * n_d, b_q * n_d, b_w * n_h, b_f * n_d
    n_o, n_f2 = HD // rows_tall, F // rows_tall
    base_q = n_m
    base_h = base_q + n_q
    base_o = base_h + 2 * n_kv * H
    base_f1 = base_o + n_o
    base_f2 = base_f1 + n_f1
    scale = float(DH) ** -0.5
    assert A_x.shape == (1, 1, D) and A_wq.shape == (D, HD) and b_m == 6
    assert D % LANES == D % rows == DH % rows == HD % rows_tall == F % rows_tall == 0
    assert SK % CB == W % CB == HD % CB == F % CB == 0
    assert max(LAG) < min(RING, 2 * n_kv, n_m, n_q, n_o)

    def kernel(x_hbm, k_hbm, v_hbm, wq_hbm, wo_hbm, w1_hbm, b1_hbm, w2_hbm, c_hbm, wm_hbm,
               o_ref,
               wm_v, wq_v, k_v, v_v, wo_v, w1_v, w2_v, x_v, c_v, b1_v,
               acc_v, col_v, q_v, s_v, ob_v, sems, small_sems):

        def sem(t, step):
            return sems.at[t, step & (RING - 1)]

        def cp_weight(src, dst, base, t, i):
            return pltpu.make_async_copy(src.at[t, :, i], dst.at[i, t], sem(t, base + i))

        cp_m = functools.partial(cp_weight, wm_hbm, wm_v, 0)
        cp_q = functools.partial(cp_weight, wq_hbm, wq_v, base_q)
        cp_f1 = functools.partial(cp_weight, w1_hbm, w1_v, base_f1)
        cp_f2 = functools.partial(cp_weight, w2_hbm, w2_v, base_f2)

        def wo_run(t, i):
            j, gap = 2 * i + t, 2 * n_o // HOPS
            lap = _div(j, HOPS, 2 * n_o)
            return jnp.where(j < HOPS * gap, (j - lap * HOPS) * gap + lap, j)

        def cp_o(t, i):
            return pltpu.make_async_copy(wo_hbm.at[:, wo_run(t, i)], wo_v.at[i, t], sem(t, base_o + i))

        def cp_cache(src, dst, which, h, r, t, blk):
            return pltpu.make_async_copy(src.at[h, t, r, :, (SK - W) // CB + blk], dst.at[blk, r, t],
                                         sem(t, base_h + (2 * h + which) * n_kv + blk * n_h + r))

        cp_k = functools.partial(cp_cache, k_hbm, k_v, 0)
        cp_v = functools.partial(cp_cache, v_hbm, v_v, 1)

        def first_head(cp):
            def flat(t, i):
                blk = _div(i, n_h, n_kv)
                return cp(0, i - blk * n_h, t, blk)
            return flat

        def start(cp, t):
            return lambda i: cp(t, i).start(priority=t)

        def weight_step(streams, i, work):
            n, cp = streams[0]
            for t in QUEUES:
                cp(t, i).wait()
                work(t)
                _dispatch(i + LAG[t], LAG[t], LAG[t] + n, [(m, start(nxt, t)) for m, nxt in streams])

        def tiles(w):
            w = w.astype(F32)
            return [w[j * SUB:(j + 1) * SUB] for j in range(w.shape[0] // SUB)]

        def put_cols(v):
            for j in range(v.shape[1] // LANES):
                t = jnp.broadcast_to(v[:, j * LANES:(j + 1) * LANES], (LANES, LANES)).T
                for g in range(LANES // SUB):
                    col_v[j * (LANES // SUB) + g] = t[g * SUB:(g + 1) * SUB]

        def add_dot(acc, runs, cols):
            prods = [[w * col for w in tiles(runs[p])] for p, col in enumerate(cols)]
            return [a + _tree_sum(col) for a, col in zip(acc, zip(*prods))]

        def row_of(parts):
            return jnp.concatenate([jnp.sum(p, axis=0, keepdims=True) for p in parts], axis=1)

        def lane_sum(v):
            return jnp.broadcast_to(jnp.sum(v, axis=1, keepdims=True), (SUB, LANES))

        zero = jnp.zeros((SUB, LANES), F32)

        def dot_wide(v, ref, streams):
            nt = ref.shape[-2] // SUB
            n_blk = streams[0][0] // n_d
            put_cols(v)
            for j in range(n_blk * nt):
                acc_v[j] = zero

            def row_groups(r, _):
                cols = [col_v[j * n_d + r] for j in range(2 * RUNS)]

                def block(blk, _):
                    i = r * n_blk + blk
                    acc = [acc_v[blk * nt + j] for j in range(nt)]

                    def work(t):
                        acc[:] = add_dot(acc, ref.at[i, t], cols[t * RUNS:(t + 1) * RUNS])
                    weight_step(streams, i, work)
                    for j in range(nt):
                        acc_v[blk * nt + j] = acc[j]
                lax.fori_loop(0, n_blk, block, None)
            lax.fori_loop(0, n_d, row_groups, None)

        def dot_tall(col_ref, ref, streams, group):
            def body(i, acc):
                acc = list(acc)

                def work(t):
                    acc[:] = add_dot(acc, ref.at[i, t], [col_ref[group(t, p, i)] for p in range(RUNS_TALL)])
                weight_step(streams, i, work)
                return acc
            return row_of(lax.fori_loop(0, streams[0][0], body, [zero] * TD))

        cp_c = pltpu.make_async_copy(c_hbm, c_v, small_sems.at[0])
        cp_x = pltpu.make_async_copy(x_hbm, x_v, small_sems.at[1])
        cp_b = pltpu.make_async_copy(b1_hbm, b1_v, small_sems.at[2])

        def prime(i, _):
            for t in QUEUES:
                _dispatch(i, 0, max(LAG), [(LAG[t], start(cp_m, t))])
        lax.fori_loop(0, 2, prime, None)
        cp_c.start()
        lax.fori_loop(2, max(LAG), prime, None)
        cp_x.start()
        cp_b.start()

        cp_c.wait()
        cond = c_v[...].astype(F32)
        dot_wide(cond * jax.nn.sigmoid(cond), wm_v, [(n_m, cp_m), (n_q, cp_q)])
        sa, ca, ga, sb, cb, gb = (row_of([acc_v[b * TD + j] for j in range(TD)]) for b in range(b_m))
        cp_x.wait()
        x = x_v[0].astype(F32)

        dot_wide(_layernorm(x) * (1.0 + ca) + sa, wq_v,
                 [(n_q, cp_q), (n_kv, first_head(cp_k)), (n_kv, first_head(cp_v))])
        for j in range(HD // LANES):
            q_v[j] = jnp.broadcast_to(jnp.sum(acc_v[j], axis=0, keepdims=True) * scale, (SUB, LANES))

        diag = (lax.broadcasted_iota(jnp.int32, (SUB, LANES), 1)
                - lax.broadcasted_iota(jnp.int32, (SUB, LANES), 0))

        def put_query(h):
            for i in range(g_h):
                g = h * g_h + i
                col_v[i] = lane_sum(jnp.where(diag == (g & 15) * SUB, q_v[g >> 4], 0.0))

        def dim_group(t, r, p):
            return (t * n_h + r) * RUNS + p

        put_query(0)

        def head(h, _):
            def cache_step(which, blk, r, work):
                for t in QUEUES:
                    (cp_k, cp_v)[which](h, r, t, blk).wait()
                    work(t)
                    ahead, nr = divmod(r + LAG[t], n_h)
                    ahead += which * b_w

                    def next_head(cp):
                        return lambda b: pl.when(h + 1 < H)(lambda: cp(h + 1, nr, t, b).start(priority=t))

                    def after_last_head(b):
                        pl.when(h + 1 == H)(lambda: cp_o(t, b * n_h + nr).start(priority=t))

                    _dispatch(blk + ahead, ahead, ahead + b_w,
                              [(b_w, start(functools.partial(cp_k, h, nr), t)),
                               (b_w, start(functools.partial(cp_v, h, nr), t)),
                               (b_w, next_head(cp_k)), (b_w, next_head(cp_v))])
                    past = ahead - 2 * b_w
                    _dispatch(blk + past, past, past + b_w, [(2 * b_w, after_last_head)])

            def key_block(blk, top):
                acc = [zero] * TC
                for r in range(n_h):
                    def work(t):
                        acc[:] = add_dot(acc, k_v.at[blk, r, t], [col_v[dim_group(t, r, p)] for p in range(RUNS)])
                    cache_step(0, blk, r, work)
                for j in range(TC):
                    s = jnp.broadcast_to(jnp.sum(acc[j], axis=0, keepdims=True), (SUB, LANES))
                    s_v[blk, j] = s
                    top = jnp.maximum(top, s)
                return top
            top = lax.fori_loop(0, b_w, key_block, jnp.full((SUB, LANES), -jnp.inf, F32))
            top = jnp.max(top, axis=1, keepdims=True)
            for g in range(g_h):
                acc_v[g] = zero

            def value_block(blk, denom):
                e = [jnp.exp(s_v[blk, j] - top) for j in range(TC)]
                for r in range(n_h):
                    def work(t):
                        for p in range(RUNS):
                            acc_v[dim_group(t, r, p)] += _tree_sum(
                                w * ej for w, ej in zip(tiles(v_v[blk, r, t, p]), e))
                    cache_step(1, blk, r, work)
                return denom + _tree_sum(e)
            denom = lax.fori_loop(0, b_w, value_block, zero)

            inv = 1.0 / lane_sum(denom)
            for g in range(g_h):
                ob_v[h * g_h + g] = lane_sum(acc_v[g]) * inv
            put_query(jnp.minimum(h + 1, H - 1))
        lax.fori_loop(0, H, head, None)

        attn = dot_tall(ob_v, wo_v, [(n_o, cp_o), (n_f1, cp_f1), (n_f2, cp_f2)],
                        lambda t, p, i: p * 2 * n_o + wo_run(t, i))
        x = x + ga * attn

        dot_wide(_layernorm(x) * (1.0 + cb) + sb, w1_v, [(n_f1, cp_f1), (n_f2, cp_f2)])
        cp_b.wait()
        a = row_of([acc_v[j] for j in range(F // LANES)]) + b1_v[...].astype(F32).reshape(1, F)
        softplus = jnp.log1p(jnp.exp(-jnp.abs(a))) + jnp.where(a > 0, a, 0.0)
        put_cols(a * jnp.tanh(softplus))
        y = dot_tall(col_v, w2_v, [(n_f2, cp_f2)], lambda t, p, i: (t * RUNS_TALL + p) * n_f2 + i)
        o_ref[0] = (x + gb * y).astype(o_ref.dtype)

    def staging(steps, runs, tiles, like):
        return pltpu.VMEM((*steps, 2, runs, SUB * tiles, LANES), like.dtype)

    def planes(*lead):
        return pltpu.VMEM((*lead, SUB, LANES), F32)

    def cache_runs(cache):
        return _runs(jnp.swapaxes(cache, 2, 3).reshape(HD, SK), TC, (H, 2, n_h, RUNS))

    return pl.pallas_call(
        kernel,
        out_shape=jax.ShapeDtypeStruct(A_x.shape, A_x.dtype),
        in_specs=[pl.BlockSpec(memory_space=pl.ANY)] * 10,
        out_specs=pl.BlockSpec(memory_space=pltpu.VMEM),
        scratch_shapes=[
            staging((n_m,), RUNS, TD, w_mod),
            staging((n_q,), RUNS, TC, A_wq),
            staging((b_w, n_h), RUNS, TC, A_k_cache),
            staging((b_w, n_h), RUNS, TC, A_v_cache),
            staging((n_o,), RUNS_TALL, TD, A_wo),
            staging((n_f1,), RUNS, TC, B_w1),
            staging((n_f2,), RUNS_TALL, TD, B_w2),
            pltpu.VMEM(A_x.shape, A_x.dtype),
            pltpu.VMEM(c.shape, c.dtype),
            pltpu.VMEM(B_b1.shape, B_b1.dtype),
            planes(max(HD // LANES, b_m * TD, F // LANES, g_h)),
            planes(max(D, F, DH) // SUB),
            planes(HD // LANES),
            planes(b_w, TC),
            planes(HD // SUB),
            pltpu.SemaphoreType.DMA((2, RING)),
            pltpu.SemaphoreType.DMA((3,)),
        ],
        compiler_params=pltpu.CompilerParams(
            vmem_limit_bytes=64 * 1024 * 1024,
            disable_bounds_checks=True,
            disable_semaphore_checks=True,
        ),
    )(
        A_x,
        cache_runs(A_k_cache),
        cache_runs(A_v_cache),
        _runs(A_wq, TC, (2, RUNS)),
        _runs(A_wo, TD, (RUNS_TALL,)),
        _runs(B_w1, TC, (2, RUNS)),
        B_b1,
        _runs(B_w2, TD, (2, RUNS_TALL)),
        c,
        _runs(w_mod, TD, (2, RUNS)),
    )
```
